```python
import os as _os
_os.environ.setdefault("JAX_PLATFORMS", "cpu")
import jax
import jax.numpy as jnp

def _softmax(x, axis=-1):
    return jax.nn.softmax(x, axis=axis)
def _gelu(x):
    return jax.nn.gelu(x, approximate=True)
def _silu(x):
    return jax.nn.silu(x)
def _sigmoid(x):
    return jax.nn.sigmoid(x)
def _layernorm(x, axis=-1, eps=1e-5):
    m = jnp.mean(x, axis=axis, keepdims=True)
    v = jnp.var(x, axis=axis, keepdims=True)
    return (x - m) / jnp.sqrt(v + eps)
def _scatter_add(tgt, idx, src, axis=0):
    return tgt.at[idx].add(src)
def _segment_sum(src, seg, n):
    return jax.ops.segment_sum(src, seg, n)
class _Rng:
    def __init__(self, key):
        self._k = key
    def _next(self):
        self._k, sub = jax.random.split(self._k)
        return sub
    def normal(self, shape):
        return jax.random.normal(self._next(), shape, dtype=jnp.bfloat16)
    def randint(self, lo, hi, shape):
        return jax.random.randint(self._next(), shape, lo, hi, dtype=jnp.int32)
    def uniform(self, shape, lo=0.0, hi=1.0):
        return jax.random.uniform(self._next(), shape, jnp.bfloat16, lo, hi)
    def permutation(self, n):
        return jax.random.permutation(self._next(), n)


kernel_name = 'standalone__mha_softmax__near_ridge'

def setup_inputs():
    _rng = _Rng(jax.random.key(int.from_bytes(__import__("os").urandom(4), "little")))
    _w = (lambda a: (lambda t: t.astype(jnp.bfloat16) if jnp.issubdtype(t.dtype, jnp.floating) else t)(jnp.asarray(a)))
    B, H, Sq, Sk, D = 8, 32, 496, 512, 192
    return {
        "q": _w((lambda *s: _rng.normal(s) * 0.05)(B, H, Sq, D)),
        "k": _w((lambda *s: _rng.normal(s) * 3.2)(B, H, Sk, D)),
        "v": _w((lambda *s: _rng.normal(s) * 0.05)(B, H, Sk, D)),
    }

def reference(q, k, v):
    scale = q.shape[-1] ** -0.5
    scores = jnp.einsum("bhqd,bhkd->bhqk", q, k) * scale
    p = _softmax(scores, axis=-1)
    return jnp.einsum("bhqk,bhkd->bhqd", p, v)
```

```python
import functools

import jax
import jax.numpy as jnp
import jax.experimental.pallas as pl
import jax.experimental.pallas.tpu as pltpu


def _attn_kernel(q_ref, k_ref, v_ref, o_ref, *, heads_per_step, scale):
    for h in range(heads_per_step):
        q = q_ref[0, h]
        k = k_ref[0, h]
        v = v_ref[0, h]
        s = jax.lax.dot_general(
            q, k, (((1,), (1,)), ((), ())), preferred_element_type=jnp.float32
        )
        s = s * scale
        m = jnp.max(s, axis=-1, keepdims=True)
        p = jnp.exp(s - m)
        l = jnp.sum(p, axis=-1, keepdims=True)
        o = jnp.dot(p.astype(jnp.bfloat16), v, preferred_element_type=jnp.float32)
        o_ref[0, h] = (o / l).astype(o_ref.dtype)


@jax.jit
def pallas_standalone__mha_softmax__near_ridge_kernel(
    q: jax.Array,
    k: jax.Array,
    v: jax.Array,
):
    B, H, Sq, D = q.shape
    Sk = k.shape[2]
    hb = 4
    scale = float(D) ** -0.5
    kernel = functools.partial(_attn_kernel, heads_per_step=hb, scale=scale)
    return pl.pallas_call(
        kernel,
        grid=(B, H // hb),
        in_specs=[
            pl.BlockSpec((1, hb, Sq, D), lambda b, h: (b, h, 0, 0)),
            pl.BlockSpec((1, hb, Sk, D), lambda b, h: (b, h, 0, 0)),
            pl.BlockSpec((1, hb, Sk, D), lambda b, h: (b, h, 0, 0)),
        ],
        out_specs=pl.BlockSpec((1, hb, Sq, D), lambda b, h: (b, h, 0, 0)),
        out_shape=jax.ShapeDtypeStruct((B, H, Sq, D), q.dtype),
        compiler_params=pltpu.CompilerParams(
            dimension_semantics=("parallel", "parallel"),
            vmem_limit_bytes=96 * 1024 * 1024,
        ),
    )(q, k, v)
```

```python
import functools

import jax
import jax.numpy as jnp
import jax.experimental.pallas as pl
import jax.experimental.pallas.tpu as pltpu


def _attn_kernel(qt_ref, kt_ref, vt_ref, ot_ref, *, heads_per_step, scale):
    for h in range(heads_per_step):
        qt = qt_ref[0, h]
        kt = kt_ref[0, h]
        vt = vt_ref[0, h]
        st = jax.lax.dot_general(
            kt, qt, (((0,), (0,)), ((), ())), preferred_element_type=jnp.float32
        )
        st = st * scale
        m = jnp.max(st, axis=0, keepdims=True)
        pt = jnp.exp(st - m)
        l = jnp.sum(pt, axis=0, keepdims=True)
        ot = jnp.dot(vt, pt.astype(jnp.bfloat16), preferred_element_type=jnp.float32)
        ot_ref[0, h] = (ot / l).astype(ot_ref.dtype)


@jax.jit
def pallas_standalone__mha_softmax__near_ridge_kernel(
    q: jax.Array,
    k: jax.Array,
    v: jax.Array,
):
    B, H, Sq, D = q.shape
    Sk = k.shape[2]
    hb = 4
    scale = float(D) ** -0.5
    qt = jnp.swapaxes(q, 2, 3)
    kt = jnp.swapaxes(k, 2, 3)
    vt = jnp.swapaxes(v, 2, 3)
    kernel = functools.partial(_attn_kernel, heads_per_step=hb, scale=scale)
    ot = pl.pallas_call(
        kernel,
        grid=(B, H // hb),
        in_specs=[
            pl.BlockSpec((1, hb, D, Sq), lambda b, h: (b, h, 0, 0)),
            pl.BlockSpec((1, hb, D, Sk), lambda b, h: (b, h, 0, 0)),
            pl.BlockSpec((1, hb, D, Sk), lambda b, h: (b, h, 0, 0)),
        ],
        out_specs=pl.BlockSpec((1, hb, D, Sq), lambda b, h: (b, h, 0, 0)),
        out_shape=jax.ShapeDtypeStruct((B, H, D, Sq), q.dtype),
        compiler_params=pltpu.CompilerParams(
            dimension_semantics=("parallel", "parallel"),
            vmem_limit_bytes=96 * 1024 * 1024,
        ),
    )(qt, kt, vt)
    return jnp.swapaxes(ot, 2, 3)
```

```python
import functools

import jax
import jax.numpy as jnp
import jax.experimental.pallas as pl
import jax.experimental.pallas.tpu as pltpu

_LOG2E = 1.4426950408889634


def _attn_kernel(qt_ref, kt_ref, vt_ref, ot_ref, *, heads_per_step, scale):
    hb = heads_per_step
    d, sk = vt_ref.shape[-2:]
    ones = jnp.ones((16, sk), jnp.bfloat16)

    def scores(h):
        return jax.lax.dot_general(
            qt_ref[0, h], kt_ref[0, h], (((0,), (0,)), ((), ())),
            preferred_element_type=jnp.float32)

    s = scores(0)
    for h in range(hb):
        s_next = scores(h + 1) if h + 1 < hb else None
        m = jnp.max(s, axis=1, keepdims=True)
        p = jnp.exp2((s - m) * (scale * _LOG2E)).astype(jnp.bfloat16)
        vt_ext = jnp.concatenate([vt_ref[0, h], ones], axis=0)
        ot = jax.lax.dot_general(
            vt_ext, p, (((1,), (1,)), ((), ())),
            preferred_element_type=jnp.float32)
        l = ot[d:d + 1]
        ot_ref[0, h] = (ot[:d] * (1.0 / l)).astype(ot_ref.dtype)
        s = s_next


@jax.jit
def pallas_standalone__mha_softmax__near_ridge_kernel(
    q: jax.Array,
    k: jax.Array,
    v: jax.Array,
):
    B, H, Sq, D = q.shape
    Sk = k.shape[2]
    hb = 8
    scale = float(D) ** -0.5
    qt = jnp.swapaxes(q, 2, 3)
    kt = jnp.swapaxes(k, 2, 3)
    vt = jnp.swapaxes(v, 2, 3)
    kernel = functools.partial(_attn_kernel, heads_per_step=hb, scale=scale)
    ot = pl.pallas_call(
        kernel,
        grid=(B, H // hb),
        in_specs=[
            pl.BlockSpec((1, hb, D, Sq), lambda b, h: (b, h, 0, 0)),
            pl.BlockSpec((1, hb, D, Sk), lambda b, h: (b, h, 0, 0)),
            pl.BlockSpec((1, hb, D, Sk), lambda b, h: (b, h, 0, 0)),
        ],
        out_specs=pl.BlockSpec((1, hb, D, Sq), lambda b, h: (b, h, 0, 0)),
        out_shape=jax.ShapeDtypeStruct((B, H, D, Sq), q.dtype),
        compiler_params=pltpu.CompilerParams(
            dimension_semantics=("parallel", "parallel"),
            vmem_limit_bytes=96 * 1024 * 1024,
        ),
    )(qt, kt, vt)
    return jnp.swapaxes(ot, 2, 3)
```
